```python
import os as _os
_os.environ.setdefault("JAX_PLATFORMS", "cpu")
import jax
import jax.numpy as jnp

def _softmax(x, axis=-1):
    return jax.nn.softmax(x, axis=axis)
def _gelu(x):
    return jax.nn.gelu(x, approximate=True)
def _silu(x):
    return jax.nn.silu(x)
def _sigmoid(x):
    return jax.nn.sigmoid(x)
def _layernorm(x, axis=-1, eps=1e-5):
    m = jnp.mean(x, axis=axis, keepdims=True)
    v = jnp.var(x, axis=axis, keepdims=True)
    return (x - m) / jnp.sqrt(v + eps)
def _scatter_add(tgt, idx, src, axis=0):
    return tgt.at[idx].add(src)
def _segment_sum(src, seg, n):
    return jax.ops.segment_sum(src, seg, n)
class _Rng:
    def __init__(self, key):
        self._k = key
    def _next(self):
        self._k, sub = jax.random.split(self._k)
        return sub
    def normal(self, shape):
        return jax.random.normal(self._next(), shape, dtype=jnp.bfloat16)
    def randint(self, lo, hi, shape):
        return jax.random.randint(self._next(), shape, lo, hi, dtype=jnp.int32)
    def uniform(self, shape, lo=0.0, hi=1.0):
        return jax.random.uniform(self._next(), shape, jnp.bfloat16, lo, hi)
    def permutation(self, n):
        return jax.random.permutation(self._next(), n)


kernel_name = 'sequential_preLN__sliding_local_dilated__dense_activation_relu__prompt'

def setup_inputs():
    _rng = _Rng(jax.random.key(int.from_bytes(__import__("os").urandom(4), "little")))
    _w = (lambda a: (lambda t: t.astype(jnp.bfloat16) if jnp.issubdtype(t.dtype, jnp.floating) else t)(jnp.asarray(a)))
    def _A_setup():
        B, S, D = 1, 2048, 1024
        return {
            "x": _w((lambda *s: _rng.normal(s) * 0.05)(B, S, D)),
            "wqkv": _w((lambda *s: _rng.normal(s) * 0.05)(D, 3 * D)),
            "wo": _w((lambda *s: _rng.normal(s) * 0.05)(D, D)),
        }
    _A_in = _A_setup()

    def _B_setup():
        B, S, D, Dff = 1, 2048, 1024, 3584
        return {
            "x": _w((lambda *s: _rng.normal(s) * 0.05)(B, S, D)),
            "w1": _w((lambda *s: _rng.normal(s) * 0.05)(D, Dff)),
            "w2": _w((lambda *s: _rng.normal(s) * 0.05)(Dff, D)),
        }
    _B_in = _B_setup()

    return {
        "A_x": _A_in["x"],
        "A_wqkv": _A_in["wqkv"],
        "A_wo": _A_in["wo"],
        "B_x": _B_in["x"],
        "B_w1": _B_in["w1"],
        "B_w2": _B_in["w2"],
    }

def reference(A_x, A_wqkv, A_wo, B_x, B_w1, B_w2):
    def _A_ref(x, wqkv, wo):
        B, S, D = x.shape
        H = 32; Dh = D // H
        W, dil = 8, 2
        qkv = (lambda x, *d: x.transpose(*d))((x @ wqkv).reshape(B, S, 3, H, Dh), 2, 0, 3, 1, 4)
        q, k, v = qkv[0], qkv[1], qkv[2]
        scale = Dh ** -0.5
        pos = jnp.arange(S)
        off = jnp.arange(W) * dil
        idx = pos[:, None] - off[None, :]
        mask = idx >= 0
        idx_c = jnp.where(mask, idx, 0).reshape(-1)
        kg = k[:, :, idx_c, :].reshape(B, H, S, W, Dh)
        vg = v[:, :, idx_c, :].reshape(B, H, S, W, Dh)
        logits = jnp.einsum("bhsd,bhswd->bhsw", q, kg) * scale
        logits = jnp.where(mask[None, None, :, :], logits, -1e9)
        attn = _softmax(logits, axis=-1)
        o = jnp.einsum("bhsw,bhswd->bhsd", attn, vg)
        return (lambda x, *d: x.transpose(*d))(o, 0, 2, 1, 3).reshape(B, S, D) @ wo

    def _B_ref(x, w1, w2):
        h = jnp.einsum("bsd,df->bsf", x, w1)
        zero = jnp.zeros_like(h)
        h = jnp.maximum(h, zero)
        return jnp.einsum("bsf,fd->bsd", h, w2)

    x = A_x
    h = x + _A_ref(_layernorm(x, axis=-1), A_wqkv, A_wo)
    h2 = h + _B_ref(_layernorm(h, axis=-1), B_w1, B_w2)
    return h2
```

```python
import functools
import jax
import jax.numpy as jnp
import numpy as np
from jax import lax
import jax.experimental.pallas as pl
import jax.experimental.pallas.tpu as pltpu

D, H, DH, W, DIL, DFF = 1024, 32, 32, 8, 2, 3584
HALO = 16
EPS = 1e-5
SCALE = DH ** -0.5
LOG2E = 1.4426950408889634
NEG = -1e9
G = 8
f32, bf16, u32 = jnp.float32, jnp.bfloat16, jnp.uint32
NT = (((1,), (1,)), ((), ()))


def b2u(x):
    return pltpu.bitcast(x, jnp.uint32)


def u2b(x):
    return pltpu.bitcast(x, jnp.bfloat16)


def layernorm(xf):
    m = jnp.mean(xf, axis=-1, keepdims=True)
    xc = xf - m
    v = jnp.mean(xc * xc, axis=-1, keepdims=True)
    return xc * lax.rsqrt(v + EPS)

def chunkperm_rows(xb):
    u = pltpu.bitcast(xb, u32)
    C = u.shape[1]
    sub = lax.broadcasted_iota(jnp.int32, (8, C), 0)
    m1 = (sub & 2) == 0
    m2 = (sub & 4) == 0
    out = {}
    for gh in range(2):
        for hh in range(8):
            xs = [u[((hh * 4 + a) * 2 + gh) * 8:((hh * 4 + a) * 2 + gh) * 8 + 8] for a in range(4)]
            for bit, shift, m in ((1, 2, m1), (2, 4, m2)):
                res = list(xs)
                for a in range(4):
                    if a & bit: continue
                    x, y = xs[a], xs[a | bit]
                    res[a] = jnp.where(m, x, pltpu.roll(y, shift, 0))
                    res[a | bit] = jnp.where(m, pltpu.roll(x, 8 - shift, 0), y)
                xs = res
            for b in range(4):
                out[(gh * 4 + b, hh)] = xs[b]
    res = jnp.concatenate([out[(g, hh)] for g in range(8) for hh in range(8)], axis=0)
    return pltpu.bitcast(res, bf16)


def make(NP=256, S=2048, R=128, RA=16, T2=256, FC=512, order="qa", vmem_mb=110, interpret=False):
    T = 2 * R
    NB = S // T
    NB2 = S // T2

    def kernel(xa_ref, xb_ref, wqkv_h, wo_h, w1_h, w2_h, o_ref,
               wraw_s, wqkv_s, wo_s, wop_s, w1_s, w2_s, q_s, k_s, v_s, ln_s, ln2_s, a_s, h_s, htmp_s, sems):
        i = pl.program_id(0)
        cps = [pltpu.make_async_copy(wqkv_h.at[:, pl.ds(t * D, D)], wraw_s.at[:, pl.ds(t * D, D)], sems.at[t]) for t in range(3)]
        cp_wo = pltpu.make_async_copy(wo_h, wo_s, sems.at[3])
        cp_w1 = pltpu.make_async_copy(w1_h, w1_s, sems.at[4])
        cp_w2 = pltpu.make_async_copy(w2_h, w2_s, sems.at[5])

        def prep_qkv(t):
            for kc in range(D // 128):
                wt = wraw_s[kc * 128:(kc + 1) * 128, t * D:(t + 1) * D].T
                wqkv_s[t * D // 2:(t + 1) * D // 2, kc * 128:(kc + 1) * 128] = b2u(chunkperm_rows(wt))

        def prep_wo():
            for cc in range(D // 128):
                wop_s[:, cc * 128:(cc + 1) * 128] = b2u(chunkperm_rows(wo_s[:, cc * 128:(cc + 1) * 128]))

        def ln1(p):
            ln_s[p * R // 2:(p + 1) * R // 2, :] = b2u(layernorm(xa_ref[p * R:(p + 1) * R, :].astype(f32)).astype(bf16))

        def qkv1(p, t):
            a = u2b(ln_s[p * R // 2:(p + 1) * R // 2, :])
            r = lax.dot_general(a, u2b(wqkv_s[t * D // 2:(t + 1) * D // 2, :]), NT, preferred_element_type=f32)
            if t == 0:
                r = r * (SCALE * LOG2E)
            dst = (q_s, k_s, v_s)[t]
            off = p * R + (0 if t == 0 else HALO)
            for g in range(G):
                dst[g, off:off + R, :] = r[:, g * 128:(g + 1) * 128]

        def qkv(p):
            for t in range(3): qkv1(p, t)

        lane = lax.broadcasted_iota(jnp.int32, (RA, 128), 1)
        ix1 = lane ^ 1
        ix2 = lane ^ 2

        def attn_rows(base, r0):
            q = [q_s[g, r0:r0 + RA, :] for g in range(G)]
            Ls = []
            for w in range(W):
                s = None
                for g in range(G):
                    pr = q[g] * k_s[g, pl.ds(HALO + r0 - DIL * w, RA), :]
                    s = pr if s is None else s + pr
                s = s + jnp.take_along_axis(s, ix1, axis=1)
                s = s + jnp.take_along_axis(s, ix2, axis=1)
                if r0 < DIL * (W - 1):
                    row = lax.broadcasted_iota(jnp.int32, (RA, 128), 0) + (base + r0)
                    s = jnp.where(row >= DIL * w, s, NEG)
                Ls.append(s)
            m = functools.reduce(jnp.maximum, Ls)
            ps = [jnp.exp2(l - m) for l in Ls]
            den = functools.reduce(jnp.add, ps)
            inv = 1.0 / den
            ps = [pp * inv for pp in ps]
            for g in range(G):
                acc = None
                for w in range(W):
                    pv = ps[w] * v_s[g, pl.ds(HALO + r0 - DIL * w, RA), :]
                    acc = pv if acc is None else acc + pv
                a_s[r0 // 2:(r0 + RA) // 2, g * 128:(g + 1) * 128] = b2u(acc.astype(bf16))

        def attn(p, base):
            for r0 in range(p * R, (p + 1) * R, RA):
                attn_rows(base, r0)

        def oproj(p, base):
            rs = slice(p * R, (p + 1) * R)
            h = xb_ref[rs, :].astype(f32) + jnp.dot(a_s[rs, :], wo_s[...], preferred_element_type=f32)
            gr = pl.ds(pl.multiple_of(base + p * R, R), R) if not isinstance(base, int) else pl.ds(base + p * R, R)
            h_s[gr, :] = h
            gr2 = pl.ds(pl.multiple_of((base + p * R) // 2, R // 2), R // 2) if not isinstance(base, int) else pl.ds((base + p * R) // 2, R // 2)
            ln2_s[gr2, :] = b2u(layernorm(h).astype(bf16))

        def halo():
            for g in range(G):
                k_s[g, 0:HALO, :] = k_s[g, T:T + HALO, :]
                v_s[g, 0:HALO, :] = v_s[g, T:T + HALO, :]

        def qkv_piece(p, t, n0, NP):
            a = u2b(ln_s[p * R // 2:(p + 1) * R // 2, :])
            r = lax.dot_general(a, u2b(wqkv_s[(t * D + n0) // 2:(t * D + n0 + NP) // 2, :]), NT, preferred_element_type=f32)
            if t == 0:
                r = r * (SCALE * LOG2E)
            dst = (q_s, k_s, v_s)[t]
            off = p * R + (0 if t == 0 else HALO)
            for gg in range(NP // 128):
                dst[n0 // 128 + gg, off:off + R, :] = r[:, gg * 128:(gg + 1) * 128]

        def qkv_pieces(p):
            return [functools.partial(qkv_piece, p, t, n0, NP) for t in range(3) for n0 in range(0, D, NP)]

        def attn_groups(p, base):
            return [functools.partial(attn_rows, base, r0) for r0 in range(p * R, (p + 1) * R, RA)]

        def o_piece(p, n0):
            rs = slice(p * R, (p + 1) * R)
            cs = slice(n0, n0 + NP)
            htmp_s[rs, cs] = xb_ref[rs, cs].astype(f32) + jnp.dot(u2b(a_s[p * R // 2:(p + 1) * R // 2, :]), u2b(wop_s[:, cs]), preferred_element_type=f32)

        def o_pieces(p):
            return [functools.partial(o_piece, p, n0) for n0 in range(0, D, NP)]

        def ln2(p, base):
            rs = slice(p * R, (p + 1) * R)
            h = htmp_s[rs, :]
            gr = pl.ds(pl.multiple_of(base + p * R, R), R) if not isinstance(base, int) else pl.ds(base + p * R, R)
            h_s[gr, :] = h
            gr2 = pl.ds(pl.multiple_of((base + p * R) // 2, R // 2), R // 2) if not isinstance(base, int) else pl.ds((base + p * R) // 2, R // 2)
            ln2_s[gr2, :] = b2u(layernorm(h).astype(bf16))

        def mix(xs, ys):
            n, m = len(xs), len(ys)
            out = []
            ia = ib = 0
            while ia < n or ib < m:
                if ib >= m or (ia < n and ia * m <= ib * n):
                    out.append(xs[ia]); ia += 1
                else:
                    out.append(ys[ib]); ib += 1
            return out

        def body(base, last):
            QB, QA = qkv_pieces(1), ([] if last else qkv_pieces(0))
            AA, AB = attn_groups(0, base), attn_groups(1, base)
            OA, OB = o_pieces(0), o_pieces(1)
            L1A = [] if last else [functools.partial(ln1, 0)]
            L1B = [] if last else [functools.partial(ln1, 1)]
            L2A, L2B = [functools.partial(ln2, 0, base)], [functools.partial(ln2, 1, base)]
            HL = [] if last else [halo]
            nq = len(QA) // 2
            na = len(AB) // 2
            if last:
                seq = mix(QB, AA) + mix(OA, AB[:na]) + L2A + AB[na:] + OB + L2B
            elif order == "qa":
                seq = mix(QB, AA) + L1A + mix(OA, AB[:na]) + mix(QA[:nq], AB[na:]) + L2A + OB + mix(QA[nq:], L2B + L1B) + HL
            elif order == "qa2":
                seq = mix(QB[:8], AA) + QB[8:] + L1A + mix(OA, AB[:na]) + mix(QA[:nq], AB[na:]) + L2A + OB + mix(QA[nq:], L2B + L1B) + HL
            elif order == "qa3":
                seq = mix(QB, AA) + L1A + mix(OA + QA[:nq], AB) + L2A + QA[nq:nq + 2] + OB + mix(QA[nq + 2:], L2B + L1B) + HL
            for th in seq: th()

        @pl.when(i == 0)
        def _():
            for c in cps: c.start()
            cp_wo.start()
            for g in range(G):
                k_s[g, 0:HALO, :] = jnp.zeros((HALO, 128), f32)
                v_s[g, 0:HALO, :] = jnp.zeros((HALO, 128), f32)
            ln1(0); ln1(1)
            cps[0].wait()
            prep_qkv(0)
            cps[1].wait()
            qkv1(0, 0); prep_qkv(1)
            cps[2].wait()
            qkv1(0, 1); prep_qkv(2)
            cp_wo.wait()
            qkv1(0, 2); prep_wo()

        @pl.when(i == 1)
        def _():
            cp_w1.start()

        @pl.when(i == 2)
        def _():
            cp_w2.start()

        @pl.when((i >= 1) & (i < NB))
        def _():
            body((i - 1) * T, False)

        @pl.when(i == NB)
        def _():
            cp_w1.wait(); cp_w2.wait()
            body((NB - 1) * T, True)

        @pl.when(i > NB)
        def _():
            j = i - NB - 1
            r = pl.ds(pl.multiple_of(j * T2, T2), T2)
            a = u2b(ln2_s[pl.ds(pl.multiple_of(j * (T2 // 2), T2 // 2), T2 // 2), :])
            acc = h_s[r, :]
            for c in range(DFF // FC):
                f = jnp.dot(a, w1_s[:, c * FC:(c + 1) * FC], preferred_element_type=f32)
                f = jnp.maximum(f, 0.0).astype(bf16)
                acc = acc + jnp.dot(f, w2_s[c * FC:(c + 1) * FC, :], preferred_element_type=f32)
            o_ref[...] = acc.astype(bf16)

    def run(A_x, A_wqkv, A_wo, B_x, B_w1, B_w2):
        x2 = A_x.reshape(S, D)
        out = pl.pallas_call(
            kernel,
            grid=(NB + 1 + NB2,),
            in_specs=[pl.BlockSpec((T, D), lambda i: (jnp.minimum(i, NB - 1), 0)),
                      pl.BlockSpec((T, D), lambda i: (jnp.clip(i - 1, 0, NB - 1), 0))] + [pl.BlockSpec(memory_space=pl.ANY)] * 4,
            out_specs=pl.BlockSpec((T2, D), lambda i: (jnp.maximum(i - NB - 1, 0), 0)),
            out_shape=jax.ShapeDtypeStruct((S, D), bf16),
            scratch_shapes=[
                pltpu.VMEM((D, 3 * D), bf16), pltpu.VMEM((3 * D // 2, D), u32), pltpu.VMEM((D, D), bf16), pltpu.VMEM((D // 2, D), u32), pltpu.VMEM((D, DFF), bf16), pltpu.VMEM((DFF, D), bf16),
                pltpu.VMEM((G, T, 128), f32), pltpu.VMEM((G, T + HALO, 128), f32), pltpu.VMEM((G, T + HALO, 128), f32),
                pltpu.VMEM((T // 2, D), u32), pltpu.VMEM((S // 2, D), u32), pltpu.VMEM((T // 2, D), u32), pltpu.VMEM((S, D), f32), pltpu.VMEM((T, D), f32),
                pltpu.SemaphoreType.DMA((6,)),
            ],
            compiler_params=pltpu.CompilerParams(dimension_semantics=("arbitrary",), vmem_limit_bytes=vmem_mb * 1024 * 1024),
            interpret=interpret,
        )(x2, x2, A_wqkv, A_wo, B_w1, B_w2)
        return out.reshape(1, S, D)
    return run


@jax.jit
def pallas_sequential_preLN__sliding_local_dilated__dense_activation_relu__prompt_kernel(
    A_x: jax.Array,
    A_wqkv: jax.Array,
    A_wo: jax.Array,
    B_x: jax.Array,
    B_w1: jax.Array,
    B_w2: jax.Array,
):
    return make()(A_x, A_wqkv, A_wo, B_x, B_w1, B_w2)
```

```python
import functools

import jax
import jax.numpy as jnp
from jax import lax
import jax.experimental.pallas as pl
import jax.experimental.pallas.tpu as pltpu

S, D, H, DH, W, DIL, DFF = 2048, 1024, 32, 32, 8, 2, 3584
G = D // 128
R = 128
T = 2 * R
NB = S // T
HALO = 16
RL = 32
NP = 256
FC = 512
CW = 256
CWS = (256, 256, 512, 512)
OSPLIT = 4
AHEAD = 3
EPS = 1e-5
SCALE = DH ** -0.5
LOG2E = 1.4426950408889634
NEG = -1e9
NT = (((1,), (1,)), ((), ()))
f32, bf16, u32 = jnp.float32, jnp.bfloat16, jnp.uint32


def b2u(x):
    return pltpu.bitcast(x, u32)


def u2b(x):
    return pltpu.bitcast(x, bf16)


def layernorm(xf):
    m = jnp.mean(xf, axis=-1, keepdims=True)
    xc = xf - m
    v = jnp.mean(xc * xc, axis=-1, keepdims=True)
    return xc * lax.rsqrt(v + EPS)


def chunk_transpose4(xs, m1, m2):
    for bit, shift, m in ((1, 2, m1), (2, 4, m2)):
        res = list(xs)
        for a in range(4):
            if a & bit:
                continue
            x, y = xs[a], xs[a | bit]
            res[a] = jnp.where(m, x, pltpu.roll(y, shift, 0))
            res[a | bit] = jnp.where(m, pltpu.roll(x, 8 - shift, 0), y)
        xs = res
    return xs


def permute_heads(xb, nh, store):
    u = pltpu.bitcast(xb, u32)
    C = u.shape[1]
    sub = lax.broadcasted_iota(jnp.int32, (8, C), 0)
    m1 = (sub & 2) == 0
    m2 = (sub & 4) == 0
    for hh in range(nh // 4):
        for gh in range(2):
            xs = [u[((hh * 4 + a) * 2 + gh) * 8:((hh * 4 + a) * 2 + gh) * 8 + 8] for a in range(4)]
            xs = chunk_transpose4(xs, m1, m2)
            for b in range(4):
                store(gh * 4 + b, hh, xs[b])


def mix(xs, ys):
    n, m = len(xs), len(ys)
    out = []
    ia = ib = 0
    while ia < n or ib < m:
        if ib >= m or (ia < n and ia * m <= ib * n):
            out.append(xs[ia])
            ia += 1
        else:
            out.append(ys[ib])
            ib += 1
    assert len(out) == n + m
    return out


def _kernel(x_h, wqkv_h, wo_h, w1_h, w2_h, o_h,
            x_s, wraw_s, wqkv_s, wo_s, wop_s, w1_s, w2_s, q_s, k_s, v_s, ln_s, ln2_s, a_s, h_s, o_s,
            wsem, xsem, fsem, osem):
    i = pl.program_id(0)
    cp_x1 = pltpu.make_async_copy(x_h.at[pl.ds(T, T), :], x_s.at[pl.ds(T, T), :], xsem.at[1])
    cp_x2 = pltpu.make_async_copy(x_h.at[pl.ds(2 * T, T), :], x_s.at[pl.ds(2 * T, T), :], xsem.at[2])
    cp_x3 = pltpu.make_async_copy(x_h.at[pl.ds(3 * T, S - 3 * T), :], x_s.at[pl.ds(3 * T, S - 3 * T), :], xsem.at[3])
    cp_x0 = [pltpu.make_async_copy(x_h.at[pl.ds(p * R, R), :], x_s.at[pl.ds(p * R, R), :], xsem.at[4 * p])
             for p in range(2)]
    wchunks = []
    for t, wd in enumerate(CWS):
        wchunks += [(t, c0, wd) for c0 in range(0, D, wd)]
    cp_wc = []
    for k, (t, c0, wd) in enumerate(wchunks):
        if t < 3:
            cs = pl.ds(t * D + c0, wd)
            cp_wc.append(pltpu.make_async_copy(wqkv_h.at[:, cs], wraw_s.at[:, cs], wsem.at[k]))
        else:
            cs = pl.ds(c0, wd)
            cp_wc.append(pltpu.make_async_copy(wo_h.at[:, cs], wo_s.at[:, cs], wsem.at[k]))
    cp_w1 = pltpu.make_async_copy(w1_h, w1_s, fsem.at[0])
    cp_w2 = pltpu.make_async_copy(w2_h, w2_s, fsem.at[1])

    def prep_w(c):
        t, cq = divmod(c, D // CW)
        nh = CW // DH
        for kc in range(D // 128):
            wt = wraw_s[kc * 128:(kc + 1) * 128, c * CW:(c + 1) * CW].T

            def store(g, hh, v):
                r = t * (D // 2) + g * 64 + (cq * (nh // 4) + hh) * 8
                wqkv_s[r:r + 8, kc * 128:(kc + 1) * 128] = v
            permute_heads(wt, nh, store)

    def prep_o(c):
        for cc in range(CW // 128):
            def store(g, hh, v):
                r = g * 64 + hh * 8
                wop_s[r:r + 8, c * CW + cc * 128:c * CW + (cc + 1) * 128] = v
            permute_heads(wo_s[:, c * CW + cc * 128:c * CW + (cc + 1) * 128], H, store)

    mres = []
    cfg = dict(gd=None, lg=None)
    never = i < 0

    def set_gates(gd, lg):
        def f():
            cfg["gd"], cfg["lg"] = gd, lg
        return [f]

    def gate_rows(xf, n):
        lg = cfg["lg"]
        if lg is not None and len(mres) > lg:
            g0 = mres[len(mres) - 1 - lg]
            return jnp.where(never, jnp.concatenate([g0[0:n, :]] * G, axis=1), xf)
        return xf

    def ln1_rows(xv, r0):
        xf = gate_rows(xv[r0:r0 + RL, :].astype(f32), RL)
        ln_s[r0 // 2:(r0 + RL) // 2, :] = b2u(layernorm(xf).astype(bf16))

    def ln1_groups(p, xv):
        return [functools.partial(ln1_rows, xv, r0) for r0 in range(p * R, (p + 1) * R, RL)]

    def ln2_rows(hv, l2v, r0):
        h = gate_rows(hv[r0:r0 + RL, :], RL)
        l2v[r0 // 2:(r0 + RL) // 2, :] = b2u(layernorm(h).astype(bf16))

    def ln2_groups(hv, l2v):
        return [functools.partial(ln2_rows, hv, l2v, r0) for r0 in range(0, T, RL)]

    def qkv_piece(p, t, n0):
        a = u2b(ln_s[p * R // 2:(p + 1) * R // 2, :])
        r = lax.dot_general(a, u2b(wqkv_s[(t * D + n0) // 2:(t * D + n0 + NP) // 2, :]), NT,
                            preferred_element_type=f32)
        if t == 0:
            r = r * (SCALE * LOG2E)
        dst = (q_s, k_s, v_s)[t]
        off = p * R + (0 if t == 0 else HALO)
        for gg in range(NP // 128):
            dst[n0 // 128 + gg, off:off + R, :] = r[:, gg * 128:(gg + 1) * 128]
        mres.append(r[0:RL, 0:128])

    def qkv_pieces(p, ts=(0, 1, 2)):
        return [functools.partial(qkv_piece, p, t, n0) for t in ts for n0 in range(0, D, NP)]

    def attn_rows(base, r0, ra):
        lane = lax.broadcasted_iota(jnp.int32, (ra, 128), 1)
        ix1 = lane ^ 1
        ix2 = lane ^ 2
        q = [q_s[g, r0:r0 + ra, :] for g in range(G)]
        gd = cfg["gd"]
        if gd is not None and len(mres) > gd:
            gate = mres[len(mres) - 1 - gd][0:ra, :]
            q = [jnp.where(never, gate, qq) for qq in q]

        def taps(ref, g):
            res = [None] * W
            for w in range(W // 2):
                both = ref[g, pl.ds(HALO + r0 - DIL * w - 8, ra + 8), :]
                res[w] = both[8:]
                res[w + W // 2] = both[:ra]
            return res
        ss = [None] * W
        for g in range(G):
            kk = taps(k_s, g)
            for w in range(W):
                pr = q[g] * kk[w]
                ss[w] = pr if ss[w] is None else ss[w] + pr
        Ls = []
        for w in range(W):
            s = ss[w]
            s = s + jnp.take_along_axis(s, ix1, axis=1)
            s = s + jnp.take_along_axis(s, ix2, axis=1)
            if isinstance(base, int) and base + r0 < DIL * (W - 1):
                row = lax.broadcasted_iota(jnp.int32, (ra, 128), 0) + (base + r0)
                s = jnp.where(row >= DIL * w, s, NEG)
            Ls.append(s)
        m = functools.reduce(jnp.maximum, Ls)
        ps = [jnp.exp2(l - m) for l in Ls]
        den = functools.reduce(jnp.add, ps)
        inv = 1.0 / den
        ps = [pp * inv for pp in ps]
        for g in range(G):
            vv = taps(v_s, g)
            acc = None
            for w in range(W):
                pv = ps[w] * vv[w]
                acc = pv if acc is None else acc + pv
            a_s[r0 // 2:(r0 + ra) // 2, g * 128:(g + 1) * 128] = b2u(acc.astype(bf16))

    def attn_groups(p, base, ra):
        return [functools.partial(attn_rows, base, r0, ra) for r0 in range(p * R, (p + 1) * R, ra)]

    def o_piece(p, n0, xc, hv):
        rs = slice(p * R, (p + 1) * R)
        cs = slice(n0, n0 + NP)
        r = jnp.dot(u2b(a_s[p * R // 2:(p + 1) * R // 2, :]), u2b(wop_s[:, cs]), preferred_element_type=f32)
        hv[rs, cs] = xc[rs, cs].astype(f32) + r
        mres.append(r[0:RL, 0:128])

    def o_pieces(p, xc, hv):
        return [functools.partial(o_piece, p, n0, xc, hv) for n0 in range(0, D, NP)]

    def halo():
        for g in range(G):
            k_s[g, 0:HALO, :] = k_s[g, T:T + HALO, :]
            v_s[g, 0:HALO, :] = v_s[g, T:T + HALO, :]

    def body(m, last):
        del mres[:]
        base = m * T
        b1 = base if isinstance(base, int) else pl.multiple_of(base, T)
        xc, hv = x_s.at[pl.ds(b1, T), :], h_s.at[pl.ds(b1, T), :]
        OA, OB = o_pieces(0, xc, hv), o_pieces(1, xc, hv)
        if last:
            AB = attn_groups(1, base, 16)
            L20 = ln2_groups(h_s.at[pl.ds(0, T), :], ln2_s.at[pl.ds(0, T // 2), :])
            seq = set_gates(None, 0) + mix(OA, mix(AB, L20[:4])) + mix(OB, L20[4:])
        else:
            xn = x_s.at[pl.ds(pl.multiple_of(base + T, T), T), :]
            xn2 = x_s.at[pl.ds(pl.multiple_of(jnp.minimum(m + 2, NB - 1) * T, T), T), :]
            QA, QB = qkv_pieces(0), qkv_pieces(1)
            AB, AA = attn_groups(1, base, 8), attn_groups(0, base + T, 8)
            L1B, L1A = ln1_groups(1, xn), ln1_groups(0, xn2)
            X = set_gates(1, None) + mix(OA + QA, mix(AB, L1B))
            Y = set_gates(0, 1) + mix(QB[:4] + OB + QB[4:], AA + L1A)
            seq = [halo] + X + Y
        for th in seq:
            th()

    @pl.when(i == 0)
    def _():
        byt = lambda t: [cp_wc[k] for k, ch in enumerate(wchunks) if ch[0] == t]
        L = [cp_x0[0]] + byt(0) + [cp_x0[1]] + byt(1) + byt(2) + byt(3) + [cp_x1, cp_x2]
        st = dict(started=0, waited=set())

        def start_more(n):
            while st["started"] < min(n, len(L)):
                L[st["started"]].start()
                st["started"] += 1

        def wait(cp):
            k = [id(c) for c in L].index(id(cp))
            start_more(k + 1)
            assert k not in st["waited"]
            st["waited"].add(k)
            cp.wait()
            start_more(len(st["waited"]) + AHEAD)

        start_more(AHEAD)
        for g in range(G):
            k_s[g, 0:HALO, :] = jnp.zeros((HALO, 128), f32)
            v_s[g, 0:HALO, :] = jnp.zeros((HALO, 128), f32)
        wait(cp_x0[0])
        x0 = x_s.at[pl.ds(0, T), :]
        for th in ln1_groups(0, x0):
            th()
        del mres[:]
        for t in range(4):
            chs = [(k, ch) for k, ch in enumerate(wchunks) if ch[0] == t]
            L1 = []
            if t == 0:
                mm = []
            elif t == 1:
                wait(cp_x0[1])
                for th in mix(qkv_pieces(0, (0,)), ln1_groups(1, x0)):
                    th()
                mm = qkv_pieces(1, (0,))
            elif t == 2:
                mm = [th for pair in zip(qkv_pieces(0, (1,)), qkv_pieces(1, (1,))) for th in pair]
                assert len(mm) == 2 * (D // NP)
                for th in mm[:2]:
                    th()
                mm = mm[2:]
            else:
                A0, L1 = attn_groups(0, 0, 16), ln1_groups(0, x_s.at[pl.ds(T, T), :])
                mm = qkv_pieces(0, (2,)) + A0[:4] + mix(qkv_pieces(1, (2,)), A0[4:] + L1)
            n = len(chs)
            bounds = [len(mm) * c // n for c in range(n + 1)]
            assert all(mm.index(th) >= bounds[n - 1] for th in L1)
            for c, (k, (tt, c0, wd)) in enumerate(chs):
                wait(cp_wc[k])
                if t == 3 and c == n - 1:
                    wait(cp_x1)
                prep = (lambda cc: prep_w(tt * (D // CW) + cc)) if tt < 3 else prep_o
                preps = [functools.partial(prep, cc) for cc in range(c0 // CW, (c0 + wd) // CW)]
                for th in mix(mm[bounds[c]:bounds[c + 1]], preps):
                    th()
        start_more(len(L))
        assert st["started"] == len(L) and len(st["waited"]) == len(L) - 1

    @pl.when(i == 1)
    def _():
        cp_x2.wait()
        cp_x3.start()

    @pl.when(i == 2)
    def _():
        cp_x3.wait()
        cp_w1.start()

    @pl.when(i == 3)
    def _():
        cp_w2.start()

    @pl.when((i >= 1) & (i < NB))
    def _():
        body(i - 1, False)

    @pl.when(i == NB)
    def _():
        cp_w1.wait()
        cp_w2.wait()
        body(NB - 1, True)

    def out_copy(j, n):
        r = pl.ds(j * T if isinstance(j, int) else pl.multiple_of(j * T, T), T)
        cs = pl.ds(n * (D // OSPLIT), D // OSPLIT)
        return pltpu.make_async_copy(o_s.at[r, cs], o_h.at[r, cs], osem.at[0])

    def p2(j, _):
        del mres[:]
        cfg["gd"], cfg["lg"] = None, 0
        jn = jnp.minimum(j + 1, NB - 1)
        L2 = ln2_groups(h_s.at[pl.ds(pl.multiple_of(jn * T, T), T), :],
                        ln2_s.at[pl.ds(pl.multiple_of(jn * (T // 2), T // 2), T // 2), :])
        a = u2b(ln2_s[pl.ds(pl.multiple_of(j * (T // 2), T // 2), T // 2), :])
        rr = pl.ds(pl.multiple_of(j * T, T), T)
        acc = h_s[rr, :]
        nch = DFF // FC
        for c in range(nch):
            f = jnp.dot(a, w1_s[:, c * FC:(c + 1) * FC], preferred_element_type=f32)
            f = jnp.maximum(f, 0.0).astype(bf16)
            if c < nch - 1:
                r2 = jnp.dot(f, w2_s[c * FC:(c + 1) * FC, :], preferred_element_type=f32)
                mres.append(r2[0:RL, 0:128])
                acc = acc + r2
            else:
                for n in range(OSPLIT):
                    cs = slice(n * (D // OSPLIT), (n + 1) * (D // OSPLIT))
                    rn = jnp.dot(f, w2_s[c * FC:(c + 1) * FC, cs], preferred_element_type=f32)
                    o_s[rr, cs] = (acc[:, cs] + rn).astype(bf16)
                    out_copy(j, n).start()
            for th in L2[len(L2) * c // nch:len(L2) * (c + 1) // nch]:
                th()

    @pl.when(i == NB)
    def _():
        lax.fori_loop(0, NB, p2, None)
        for j in range(NB):
            for n in range(OSPLIT):
                out_copy(j, n).wait()


@jax.jit
def pallas_sequential_preLN__sliding_local_dilated__dense_activation_relu__prompt_kernel(
    A_x: jax.Array,
    A_wqkv: jax.Array,
    A_wo: jax.Array,
    B_x: jax.Array,
    B_w1: jax.Array,
    B_w2: jax.Array,
):
    out = pl.pallas_call(
        _kernel,
        grid=(NB + 1,),
        in_specs=[pl.BlockSpec(memory_space=pl.ANY)] * 5,
        out_specs=pl.BlockSpec(memory_space=pl.ANY),
        out_shape=jax.ShapeDtypeStruct((S, D), bf16),
        scratch_shapes=[
            pltpu.VMEM((S, D), bf16),
            pltpu.VMEM((D, 3 * D), bf16), pltpu.VMEM((3 * D // 2, D), u32),
            pltpu.VMEM((D, D), bf16), pltpu.VMEM((D // 2, D), u32),
            pltpu.VMEM((D, DFF), bf16), pltpu.VMEM((DFF, D), bf16),
            pltpu.VMEM((G, T, 128), f32),
            pltpu.VMEM((G, T + HALO, 128), f32), pltpu.VMEM((G, T + HALO, 128), f32),
            pltpu.VMEM((T // 2, D), u32), pltpu.VMEM((S // 2, D), u32),
            pltpu.VMEM((T // 2, D), u32),
            pltpu.VMEM((S, D), f32), pltpu.VMEM((S, D), bf16),
            pltpu.SemaphoreType.DMA((sum(D // wd for wd in CWS),)),
            pltpu.SemaphoreType.DMA((5,)),
            pltpu.SemaphoreType.DMA((2,)),
            pltpu.SemaphoreType.DMA((1,)),
        ],
        compiler_params=pltpu.CompilerParams(
            dimension_semantics=("arbitrary",), vmem_limit_bytes=110 * 1024 * 1024),
    )(A_x.reshape(S, D), A_wqkv, A_wo, B_w1, B_w2)
    return out.reshape(1, S, D)
```
